```python
import jax
import jax.numpy as jnp

def _softmax(x, axis=-1):
    return jax.nn.softmax(x, axis=axis)
def _gelu(x):
    return jax.nn.gelu(x, approximate=True)
def _silu(x):
    return jax.nn.silu(x)
def _sigmoid(x):
    return jax.nn.sigmoid(x)
def _layernorm(x, axis=-1, eps=1e-5):
    m = jnp.mean(x, axis=axis, keepdims=True)
    v = jnp.var(x, axis=axis, keepdims=True)
    return (x - m) / jnp.sqrt(v + eps)
def _scatter_add(tgt, idx, src, axis=0):
    return tgt.at[idx].add(src)
def _segment_sum(src, seg, n):
    return jax.ops.segment_sum(src, seg, n)
class _Rng:
    def __init__(self, key):
        self._k = key
    def _next(self):
        self._k, sub = jax.random.split(self._k)
        return sub
    def normal(self, shape):
        return jax.random.normal(self._next(), shape, dtype=jnp.bfloat16)
    def randint(self, lo, hi, shape):
        return jax.random.randint(self._next(), shape, lo, hi, dtype=jnp.int32)
    def uniform(self, shape, lo=0.0, hi=1.0):
        return jax.random.uniform(self._next(), shape, jnp.bfloat16, lo, hi)
    def permutation(self, n):
        return jax.random.permutation(self._next(), n)


kernel_name = 'recurrent_scan__sliding_block_cached__moe_arch_mod__prompt'

def setup_inputs():
    _rng = _Rng(jax.random.key(int.from_bytes(__import__("os").urandom(4), "little")))
    _w = (lambda a: (lambda t: t.astype(jnp.bfloat16) if jnp.issubdtype(t.dtype, jnp.floating) else t)(jnp.asarray(a)))
    def _A_setup():
        B, Sq, D = 1, 2048, 640
        Hq, Hkv, Sk, Dh = 32, 32, 2048, 192
        assert Hq % Hkv == 0, (Hq, Hkv)
        return {
            "x": _w((lambda *s: _rng.normal(s) * 0.05)(B, Sq, D)),
            "k_cache": _w((lambda *s: _rng.normal(s) * 0.05)(B, Hkv, Sk, Dh)),
            "v_cache": _w((lambda *s: _rng.normal(s) * 0.05)(B, Hkv, Sk, Dh)),
            "wq": _w((lambda *s: _rng.normal(s) * 0.05)(D, Hq * Dh) * (D ** -0.5)),
            "wo": _w((lambda *s: _rng.normal(s) * 0.05)(Hq * Dh, D) * ((Hq * Dh) ** -0.5)),
        }
    _A_in = _A_setup()

    def _B_setup():
        B, S, D, F, C = 1, 2048, 640, 1536, 2
        return {
            "x": _w((lambda *s: _rng.normal(s) * 0.05)(B, S, D)),
            "w_r": _w((lambda *s: _rng.normal(s) * 0.05)(D)),
            "w_gate": _w((lambda *s: _rng.normal(s) * 0.05)(D, F)),
            "w_up": _w((lambda *s: _rng.normal(s) * 0.05)(D, F)),
            "w_down": _w((lambda *s: _rng.normal(s) * 0.05)(F, D)),
        }
    _B_in = _B_setup()

    return {
        "A_x": _A_in["x"],
        "A_k_cache": _A_in["k_cache"],
        "A_v_cache": _A_in["v_cache"],
        "A_wq": _A_in["wq"],
        "A_wo": _A_in["wo"],
        "B_x": _B_in["x"],
        "B_w_r": _B_in["w_r"],
        "B_w_gate": _B_in["w_gate"],
        "B_w_up": _B_in["w_up"],
        "B_w_down": _B_in["w_down"],
    }

def reference(A_x, A_k_cache, A_v_cache, A_wq, A_wo, B_x, B_w_r, B_w_gate, B_w_up, B_w_down):
    def _A_ref(x, k_cache, v_cache, wq, wo):
        B, Sq, D = x.shape
        Hq, Dh = 32, 192
        Hkv, Sk = k_cache.shape[1], k_cache.shape[2]
        W = min(4096, max(256, Sk // 4))
        rep = Hq // Hkv
        q = (lambda x, *d: x.transpose(*d))((x @ wq).reshape(B, Sq, Hq, Dh), 0, 2, 1, 3)
        k = jnp.repeat(k_cache[:, :, Sk - W:, :], rep, axis=1)
        v = jnp.repeat(v_cache[:, :, Sk - W:, :], rep, axis=1)
        scores = jnp.einsum("bhqd,bhkd->bhqk", q, k) * (Dh ** -0.5)
        p = _softmax(scores, axis=-1)
        o = jnp.einsum("bhqk,bhkd->bhqd", p, v)
        return (lambda x, *d: x.transpose(*d))(o, 0, 2, 1, 3).reshape(B, Sq, Hq * Dh) @ wo

    def _B_ref(x, w_r, w_gate, w_up, w_down):
        B, S, D = x.shape
        C = 2
        r = x @ w_r
        idx = jnp.argsort(-r, axis=-1)[:, :C]
        idx_e = jnp.repeat(idx.reshape(B, C, 1), D, axis=2)
        x_sel = jnp.take_along_axis(x, idx_e, axis=1)
        g = _silu(x_sel @ w_gate)
        u = x_sel @ w_up
        y = (g * u) @ w_down
        r_sel = _sigmoid(jnp.take_along_axis(r, idx, axis=1))
        y = y * r_sel.reshape(B, C, 1)
        b_off = (jnp.arange(B) * S).reshape(B, 1)
        flat_idx = (idx + b_off).reshape(B * C)
        zero = (x * 0.0).reshape(B * S, D)
        upd = _scatter_add(zero, flat_idx, y.reshape(B * C, D), axis=0)
        return x + upd.reshape(B, S, D)

    x = A_x
    xn = _layernorm(x, axis=-1)
    s = _A_ref(xn, A_k_cache, A_v_cache, A_wq, A_wo)
    g = _silu(_B_ref(xn, B_w_r, B_w_gate, B_w_up, B_w_down))
    return x + s * g
```

```python
import numpy as np
import jax
import jax.numpy as jnp
from jax import lax
import jax.experimental.pallas as pl
import jax.experimental.pallas.tpu as pltpu

_NT = (((1,), (1,)), ((), ()))
_BF = jnp.bfloat16
_F32 = jnp.float32


@jax.jit
def pallas_recurrent_scan__sliding_block_cached__moe_arch_mod__prompt_kernel(
    A_x: jax.Array,
    A_k_cache: jax.Array,
    A_v_cache: jax.Array,
    A_wq: jax.Array,
    A_wo: jax.Array,
    B_x: jax.Array,
    B_w_r: jax.Array,
    B_w_gate: jax.Array,
    B_w_up: jax.Array,
    B_w_down: jax.Array,
):
    del B_x
    _, S, D = A_x.shape
    H, DH = 32, 192
    SK = A_k_cache.shape[2]
    W = min(4096, max(256, SK // 4))
    F = B_w_gate.shape[1]
    NP = H // 2
    BQ = 512
    NQ = S // BQ
    GR = S // NP
    LNR = 128
    qscale = float(DH ** -0.5 * np.log2(np.e))
    eps = float(np.asarray(1e-5, np.float32).astype(jnp.bfloat16).astype(np.float32))

    def rb(a):
        return a.astype(_BF).astype(_F32)

    def silu(a):
        return a * (1.0 / (1.0 + jnp.exp(-a)))

    def kernel(x_ref, kt_ref, vt_ref, wq_ref, wo_ref, wr_ref, wg_hbm, wu_hbm, wd_hbm,
               o_ref, xn_s, g_s, acc_s, kp_s, wot_s, r_s, y_s, idx_s, wg_s, wu_s, wd_s, sem):
        p = pl.program_id(0)

        def ffn_copies():
            return (pltpu.make_async_copy(wg_hbm, wg_s, sem.at[0]),
                    pltpu.make_async_copy(wu_hbm, wu_s, sem.at[1]),
                    pltpu.make_async_copy(wd_hbm, wd_s, sem.at[2]))

        @pl.when(p == 0)
        def _():
            for c in ffn_copies():
                c.start()
            wr = wr_ref[...].astype(_F32)

            def ln(i, carry):
                r = pl.ds(pl.multiple_of(i * LNR, LNR), LNR)
                x = x_ref[r, :].astype(_F32)
                m = jnp.mean(x, axis=-1, keepdims=True)
                xc = x - m
                v = jnp.mean(xc * xc, axis=-1, keepdims=True)
                sd = rb(jnp.sqrt(rb(rb(v) + eps)))
                xn = (rb(x - rb(m)) / sd).astype(_BF)
                xn_s[r, :] = xn
                r_s[r, :] = rb(jnp.sum(xn.astype(_F32) * wr, axis=-1, keepdims=True))
                return carry

            lax.fori_loop(0, S // LNR, ln, 0)
            acc_s[...] = jnp.zeros_like(acc_s)

        @pl.when(p == 1)
        def _():
            r = r_s[...]
            rows = lax.broadcasted_iota(jnp.int32, (S, 1), 0)
            m1 = jnp.max(r)
            i1 = jnp.min(jnp.where(r == m1, rows, S - 1))
            other = rows != i1
            m2 = jnp.max(jnp.where(other, r, -jnp.inf))
            i2 = jnp.min(jnp.where(other & (r == m2), rows, S - 1))
            idx_s[0] = i1
            idx_s[1] = i2
            sub = lax.broadcasted_iota(jnp.int32, (16, D), 0)
            grp = []
            for i in (i1, i2):
                base = pl.multiple_of((i // 16) * 16, 16)
                blk = xn_s[pl.ds(base, 16), :]
                grp.append(jnp.where(sub == i - base, blk, jnp.zeros_like(blk)))
            xs = jnp.concatenate(grp, axis=0)
            for c in ffn_copies():
                c.wait()
            gate = rb(silu(rb(jnp.dot(xs, wg_s[...], preferred_element_type=_F32))))
            up = rb(jnp.dot(xs, wu_s[...], preferred_element_type=_F32))
            hid = (gate * up).astype(_BF)
            y = rb(jnp.dot(hid, wd_s[...], preferred_element_type=_F32))
            for k, m in enumerate((m1, m2)):
                wsel = rb(1.0 / (1.0 + jnp.exp(-jnp.full((16, D), m, _F32))))
                y_s[k * 16:(k + 1) * 16, :] = rb(y[k * 16:(k + 1) * 16] * wsel)

        gr = pl.ds(pl.multiple_of(p * GR, GR), GR)
        g_s[gr, :] = silu(xn_s[gr, :].astype(_F32)).astype(_BF)

        z = jnp.zeros((256 - DH, W), _BF)
        kp_s[0] = jnp.concatenate([kt_ref[0], z], axis=0)
        kp_s[1] = jnp.concatenate([z, kt_ref[1]], axis=0)
        wot_s[...] = wo_ref[...].T

        for j in range(NQ):
            r = pl.ds(j * BQ, BQ)
            q2 = jnp.dot(xn_s[r, :], wq_ref[...], preferred_element_type=_F32)
            q2 = (q2 * qscale).astype(_BF)
            qs = (q2[:, 0:256], q2[:, 128:384])
            ss = [jnp.dot(qs[h], kp_s[h], preferred_element_type=_F32) for h in range(2)]
            ots = []
            for h, s in enumerate(ss):
                e = jnp.exp2(s - jnp.max(s, axis=1, keepdims=True))
                pr = (e * (1.0 / jnp.sum(e, axis=1, keepdims=True))).astype(_BF)
                ot = lax.dot_general(vt_ref[h], pr, _NT, preferred_element_type=_F32)
                ots.append(ot.astype(_BF))
            ot = jnp.concatenate(ots, axis=0)
            acc_s[:, r] += jnp.dot(wot_s[...], ot, preferred_element_type=_F32)

        @pl.when(p == NP - 1)
        def _():
            sub = lax.broadcasted_iota(jnp.int32, (16, D), 0)
            for k in range(2):
                i = idx_s[k]
                base = pl.multiple_of((i // 16) * 16, 16)
                rs = pl.ds(base, 16)
                zr = rb(xn_s[rs, :].astype(_F32) + y_s[k * 16:(k + 1) * 16, :])
                g_s[rs, :] = jnp.where(sub == i - base, silu(zr).astype(_BF), g_s[rs, :])
            for j in range(NQ):
                r = pl.ds(j * BQ, BQ)
                s = rb(acc_s[:, r].T)
                sg = rb(s * g_s[r, :].astype(_F32))
                o_ref[r, :] = (x_ref[r, :].astype(_F32) + sg).astype(o_ref.dtype)

    def hbm(a):
        return pltpu.with_memory_space_constraint(a, pltpu.HBM)

    kt = jnp.swapaxes(A_k_cache, 2, 3)
    vt = jnp.swapaxes(A_v_cache, 2, 3)
    wb = SK // W - 1
    any_spec = pl.BlockSpec(memory_space=pl.ANY)
    return pl.pallas_call(
        kernel,
        grid=(NP,),
        in_specs=[
            pl.BlockSpec((None, S, D), lambda p: (0, 0, 0)),
            pl.BlockSpec((None, 2, DH, W), lambda p: (0, p, 0, wb)),
            pl.BlockSpec((None, 2, DH, W), lambda p: (0, p, 0, wb)),
            pl.BlockSpec((D, 2 * DH), lambda p: (0, p)),
            pl.BlockSpec((2 * DH, D), lambda p: (p, 0)),
            pl.BlockSpec((1, D), lambda p: (0, 0)),
            any_spec, any_spec, any_spec,
        ],
        out_specs=pl.BlockSpec((None, S, D), lambda p: (0, 0, 0)),
        out_shape=jax.ShapeDtypeStruct((1, S, D), A_x.dtype),
        scratch_shapes=[
            pltpu.VMEM((S, D), _BF),
            pltpu.VMEM((S, D), _BF),
            pltpu.VMEM((D, S), _F32),
            pltpu.VMEM((2, 256, W), _BF),
            pltpu.VMEM((D, 2 * DH), _BF),
            pltpu.VMEM((S, 1), _F32),
            pltpu.VMEM((32, D), _F32),
            pltpu.SMEM((2,), jnp.int32),
            pltpu.VMEM((D, F), _BF),
            pltpu.VMEM((D, F), _BF),
            pltpu.VMEM((F, D), _BF),
            pltpu.SemaphoreType.DMA((3,)),
        ],
        compiler_params=pltpu.CompilerParams(
            dimension_semantics=("arbitrary",), vmem_limit_bytes=100 * 2**20),
        name="mykernel",
    )(hbm(A_x), hbm(kt), hbm(vt), hbm(A_wq), hbm(A_wo), hbm(B_w_r.reshape(1, D)),
      hbm(B_w_gate), hbm(B_w_up), hbm(B_w_down))
```

```python
import contextlib
import numpy as np
import jax
import jax.numpy as jnp
from jax import lax
import jax.experimental.pallas as pl
import jax.experimental.pallas.tpu as pltpu

_NT = (((1,), (1,)), ((), ()))
_BF = jnp.bfloat16
_F32 = jnp.float32
_IMIN = -2 ** 31


@jax.jit
def pallas_recurrent_scan__sliding_block_cached__moe_arch_mod__prompt_kernel(
    A_x: jax.Array,
    A_k_cache: jax.Array,
    A_v_cache: jax.Array,
    A_wq: jax.Array,
    A_wo: jax.Array,
    B_x: jax.Array,
    B_w_r: jax.Array,
    B_w_gate: jax.Array,
    B_w_up: jax.Array,
    B_w_down: jax.Array,
):
    cfg = dict(LNU=2)
    del B_x
    _, S, D = A_x.shape
    H, DH = 32, 192
    SK = A_k_cache.shape[2]
    W = min(4096, max(256, SK // 4))
    F = B_w_gate.shape[1]
    NP = H // 2
    PW = 2 * DH
    BQ = 512
    NQ = S // BQ
    LNR = cfg.get("LNR", 128)
    FR = cfg.get("FR", 128)
    qscale = float(DH ** -0.5 * np.log2(np.e))
    eps = float(np.asarray(1e-5, np.float32).astype(jnp.bfloat16).astype(np.float32))
    scope = lambda n: contextlib.nullcontext()

    def rb(a):
        return a.astype(_BF).astype(_F32)

    def sigmoid(a):
        return 0.5 * jnp.tanh(0.5 * a) + 0.5

    def silu(a):
        h = 0.5 * a
        return h * jnp.tanh(h) + h

    def kernel(x_hbm, kt_hbm, vt_hbm, wq_hbm, wo_hbm, wr_hbm, wg_hbm, wu_hbm, wd_hbm, o_hbm,
               x_s, xn_s, g_s, o_s, acc_s, kp_s, vt_s, wq_s, wo_s, wot_s, wr_s,
               wg_s, wu_s, wd_s, xsem, psem, fsem, osem):

        def x_copy(j):
            return pltpu.make_async_copy(x_hbm.at[0, pl.ds(j * BQ, BQ), :], x_s.at[pl.ds(j * BQ, BQ), :], xsem.at[j])

        def o_copy(j):
            return pltpu.make_async_copy(o_s.at[pl.ds(j * BQ, BQ), :], o_hbm.at[0, pl.ds(j * BQ, BQ), :], osem.at[j])

        def pair_copies(p, slot):
            win = pl.ds(SK - W, W)
            c0 = pl.multiple_of(p * PW, 128)
            return (
                pltpu.make_async_copy(wq_hbm.at[:, pl.ds(c0, PW)], wq_s.at[slot], psem.at[slot, 0]),
                pltpu.make_async_copy(kt_hbm.at[0, 2 * p, :, win], kp_s.at[slot, 0, pl.ds(0, DH), :], psem.at[slot, 1]),
                pltpu.make_async_copy(kt_hbm.at[0, 2 * p + 1, :, win], kp_s.at[slot, 1, pl.ds(256 - DH, DH), :], psem.at[slot, 2]),
                pltpu.make_async_copy(vt_hbm.at[0, pl.ds(2 * p, 2), :, win], vt_s.at[slot], psem.at[slot, 3]),
                pltpu.make_async_copy(wo_hbm.at[pl.ds(c0, PW), :], wo_s.at[slot], psem.at[slot, 4]),
            )

        def ffn_copies():
            return (pltpu.make_async_copy(wg_hbm, wg_s, fsem.at[0]),
                    pltpu.make_async_copy(wu_hbm, wu_s, fsem.at[1]),
                    pltpu.make_async_copy(wd_hbm, wd_s, fsem.at[2]))

        wr_copy = pltpu.make_async_copy(wr_hbm, wr_s, fsem.at[3])

        def layernorm(j, top):
            wr = wr_s[...].astype(_F32).reshape(1, D)

            def slab(i, top):
                t1, t2 = top
                r0 = pl.multiple_of(j * BQ + i * LNR, LNR)
                r = pl.ds(r0, LNR)
                x = x_s[r, :].astype(_F32)
                m = jnp.sum(x, axis=-1, keepdims=True) * (1.0 / D)
                xc = x - m
                v = rb(rb(jnp.sum(xc * xc, axis=-1, keepdims=True) * (1.0 / D)) + eps)
                inv = 1.0 / rb(v * lax.rsqrt(v))
                xn = (rb(x - rb(m)) * inv).astype(_BF)
                xn_s[r, :] = xn
                xf = xn.astype(_F32)
                g_s[r, :] = silu(xf).astype(_BF)
                sc = rb(jnp.sum(xf * wr, axis=-1, keepdims=True)) + 0.0
                bits = lax.bitcast_convert_type(sc, jnp.int32)
                key = (bits ^ ((bits >> 31) & 0x7FFFFFFF)) & -65536
                row = r0 + lax.broadcasted_iota(jnp.int32, (LNR, 1), 0)
                key = jnp.where(sc != sc, _IMIN, key | (S - 1 - row))
                for u in range(LNR // 8):
                    k = key[u * 8:(u + 1) * 8]
                    t2 = jnp.maximum(t2, jnp.minimum(t1, k))
                    t1 = jnp.maximum(t1, k)
                return t1, t2

            return lax.fori_loop(0, BQ // LNR, slab, top, unroll=cfg.get("LNU", 1))

        def route_and_ffn(top):
            t1, t2 = top
            k1 = jnp.max(t1)
            k2 = jnp.max(jnp.where(t1 == k1, t2, t1))
            i1, i2 = (S - 1 - (k & 0xFFFF) for k in (k1, k2))

            def score(k):
                kk = jnp.full((16, D), k, jnp.int32) & -65536
                return lax.bitcast_convert_type((kk ^ ((kk >> 31) & 0x7FFFFFFF)) & -65536, _F32)

            m1, m2 = score(k1), score(k2)
            sub = lax.broadcasted_iota(jnp.int32, (16, D), 0)
            grp = []
            for i in (i1, i2):
                base = pl.multiple_of((i // 16) * 16, 16)
                blk = xn_s[pl.ds(base, 16), :]
                grp.append(jnp.where(sub == i - base, blk, jnp.zeros_like(blk)))
            xs = jnp.concatenate(grp, axis=0)
            for c in ffn_copies():
                c.wait()
            gt = rb(silu(rb(jnp.dot(xs, wg_s[...], preferred_element_type=_F32))))
            up = rb(jnp.dot(xs, wu_s[...], preferred_element_type=_F32))
            hid = (gt * up).astype(_BF)
            y = rb(jnp.dot(hid, wd_s[...], preferred_element_type=_F32))
            for k, (i, m) in enumerate(((i1, m1), (i2, m2))):
                upd = rb(y[k * 16:(k + 1) * 16] * rb(sigmoid(m)))
                rs = pl.ds(pl.multiple_of((i // 16) * 16, 16), 16)
                z = rb(xn_s[rs, :].astype(_F32) + upd)
                g_s[rs, :] = jnp.where(sub == i % 16, silu(z).astype(_BF), g_s[rs, :])

        def attention_pair(slot):
            def qproj(j):
                q2 = jnp.dot(xn_s[pl.ds(j * BQ, BQ), :], wq_s[slot], preferred_element_type=_F32)
                return (q2 * qscale).astype(_BF)

            def attn(s, h):
                e = jnp.exp2(s - jnp.max(s, axis=1, keepdims=True))
                l = jnp.sum(e, axis=1, keepdims=True)
                o = lax.dot_general(vt_s[slot, h], e.astype(_BF), _NT, preferred_element_type=_F32)
                il = jnp.broadcast_to(1.0 / l, (BQ, 128)).T[0:1]
                return (o * il).astype(_BF)

            wot_s[...] = wo_s[slot].T
            q2 = qproj(0)
            for j in range(NQ):
                r = pl.ds(j * BQ, BQ)
                ss = [jnp.dot(q2[:, h * 128:h * 128 + 256], kp_s[slot, h], preferred_element_type=_F32)
                      for h in range(2)]
                ot = jnp.concatenate([attn(ss[h], h) for h in range(2)], axis=0)
                if j + 1 < NQ:
                    q2 = qproj(j + 1)
                acc_s[:, r] += jnp.dot(wot_s[...], ot, preferred_element_type=_F32)

        c0 = pair_copies(0, 0)
        wr_copy.start()
        x_copy(0).start()
        with scope('zero'):
            acc_s[...] = jnp.zeros_like(acc_s)
            zpad = jnp.zeros((256 - DH, W), _BF)
            for sl in range(2):
                kp_s[sl, 0, pl.ds(DH, 256 - DH), :] = zpad
                kp_s[sl, 1, pl.ds(0, 256 - DH), :] = zpad
        with scope('wrwait'):
            wr_copy.wait()
        top = (jnp.full((8, 1), _IMIN, jnp.int32),) * 2
        later = cfg.get("LATER", ((0,), (1, 2), (3,), (4,)))
        with scope('ln'):
            for j in range(NQ):
                x_copy(j).wait()
                if j + 1 < NQ:
                    x_copy(j + 1).start()
                for c in later[j]:
                    c0[c].start()
                top = layernorm(j, top)

        def loop(p, carry):
            slot = p % 2

            @pl.when(p + 1 < NP)
            def _():
                for c in pair_copies(p + 1, 1 - slot):
                    c.start()

            @pl.when(p == 2)
            def _():
                for c in ffn_copies():
                    c.start()

            for c in pair_copies(p, slot):
                c.wait()
            attention_pair(slot)
            return carry

        with scope('loop'):
            lax.fori_loop(0, NP, loop, 0)
        with scope('ffn'):
            route_and_ffn(top)
        with scope('fin'):
            for j in range(NQ):
                def fslab(i, carry):
                    r = pl.ds(pl.multiple_of(j * BQ + i * FR, FR), FR)
                    s = rb(acc_s[:, r].T)
                    sg = rb(s * g_s[r, :].astype(_F32))
                    o_s[r, :] = (x_s[r, :].astype(_F32) + sg).astype(o_s.dtype)
                    return carry
                lax.fori_loop(0, BQ // FR, fslab, 0, unroll=cfg.get('FU', 2))
                o_copy(j).start()
        with scope('owait'):
            for j in range(NQ):
                o_copy(j).wait()

    def hbm(a):
        return pltpu.with_memory_space_constraint(a, pltpu.HBM)

    kt = jnp.swapaxes(A_k_cache, 2, 3)
    vt = jnp.swapaxes(A_v_cache, 2, 3)
    any_spec = pl.BlockSpec(memory_space=pl.ANY)
    DMA = pltpu.SemaphoreType.DMA
    return pl.pallas_call(
        kernel,
        in_specs=[any_spec] * 9,
        out_specs=any_spec,
        out_shape=jax.ShapeDtypeStruct((1, S, D), A_x.dtype),
        scratch_shapes=[
            pltpu.VMEM((S, D), _BF),
            pltpu.VMEM((S, D), _BF),
            pltpu.VMEM((S, D), _BF),
            pltpu.VMEM((S, D), _BF),
            pltpu.VMEM((D, S), _F32),
            pltpu.VMEM((2, 2, 256, W), _BF),
            pltpu.VMEM((2, 2, DH, W), _BF),
            pltpu.VMEM((2, D, PW), _BF),
            pltpu.VMEM((2, PW, D), _BF),
            pltpu.VMEM((D, PW), _BF),
            pltpu.VMEM((D,), _BF),
            pltpu.VMEM((D, F), _BF),
            pltpu.VMEM((D, F), _BF),
            pltpu.VMEM((F, D), _BF),
            DMA((NQ,)), DMA((2, 5)), DMA((4,)), DMA((NQ,)),
        ],
        compiler_params=pltpu.CompilerParams(vmem_limit_bytes=100 * 2**20, flags=cfg.get("flags")),
        name="mykernel",
    )(hbm(A_x), hbm(kt), hbm(vt), hbm(A_wq), hbm(A_wo), hbm(B_w_r),
      hbm(B_w_gate), hbm(B_w_up), hbm(B_w_down))
```

```python
import contextlib
import numpy as np
import jax
import jax.numpy as jnp
from jax import lax
import jax.experimental.pallas as pl
import jax.experimental.pallas.tpu as pltpu

_NT = (((1,), (1,)), ((), ()))
_BF = jnp.bfloat16
_F32 = jnp.float32
_IMIN = -2 ** 31


@jax.jit
def pallas_recurrent_scan__sliding_block_cached__moe_arch_mod__prompt_kernel(
    A_x: jax.Array,
    A_k_cache: jax.Array,
    A_v_cache: jax.Array,
    A_wq: jax.Array,
    A_wo: jax.Array,
    B_x: jax.Array,
    B_w_r: jax.Array,
    B_w_gate: jax.Array,
    B_w_up: jax.Array,
    B_w_down: jax.Array,
):
    cfg = dict(LNU=2, OR=128)
    del B_x
    _, S, D = A_x.shape
    H, DH = 32, 192
    SK = A_k_cache.shape[2]
    W = min(4096, max(256, SK // 4))
    F = B_w_gate.shape[1]
    NP = H // 2
    PW = 2 * DH
    BQ = 512
    NQ = S // BQ
    OR = cfg.get('OR', 256)
    NO = S // OR
    LNR = cfg.get("LNR", 128)
    FR = cfg.get("FR", 128)
    qscale = float(DH ** -0.5 * np.log2(np.e))
    eps = float(np.asarray(1e-5, np.float32).astype(jnp.bfloat16).astype(np.float32))
    scope = lambda n: contextlib.nullcontext()

    def rb(a):
        return a.astype(_BF).astype(_F32)

    def recip(a):
        r0 = pl.reciprocal(a, approx=True)
        return r0 * (2.0 - a * r0)

    def sigmoid(a):
        return 0.5 * jnp.tanh(0.5 * a) + 0.5

    def silu(a):
        h = 0.5 * a
        return h * jnp.tanh(h) + h

    def kernel(x_hbm, kt_hbm, vt_hbm, wq_hbm, wo_hbm, wr_hbm, wg_hbm, wu_hbm, wd_hbm, o_hbm,
               x_s, xn_s, o_s, acc_s, kp_s, vt_s, wq_s, wo_s, wot_s, wr_s,
               wg_s, wu_s, wd_s, xsem, psem, fsem, osem):

        def x_copy(j):
            return pltpu.make_async_copy(x_hbm.at[0, pl.ds(j * BQ, BQ), :], x_s.at[pl.ds(j * BQ, BQ), :], xsem.at[j])

        def o_copy(j):
            return pltpu.make_async_copy(o_s.at[pl.ds(j * OR, OR), :], o_hbm.at[0, pl.ds(j * OR, OR), :], osem.at[j])

        def pair_copies(p, slot):
            win = pl.ds(SK - W, W)
            c0 = pl.multiple_of(p * PW, 128)
            return (
                pltpu.make_async_copy(wq_hbm.at[:, pl.ds(c0, PW)], wq_s.at[slot], psem.at[slot, 0]),
                pltpu.make_async_copy(kt_hbm.at[0, 2 * p, :, win], kp_s.at[slot, 0, pl.ds(0, DH), :], psem.at[slot, 1]),
                pltpu.make_async_copy(kt_hbm.at[0, 2 * p + 1, :, win], kp_s.at[slot, 1, pl.ds(256 - DH, DH), :], psem.at[slot, 2]),
                pltpu.make_async_copy(vt_hbm.at[0, pl.ds(2 * p, 2), :, win], vt_s.at[slot], psem.at[slot, 3]),
                pltpu.make_async_copy(wo_hbm.at[pl.ds(c0, PW), :], wo_s.at[slot], psem.at[slot, 4]),
            )

        def ffn_copies():
            return (pltpu.make_async_copy(wg_hbm, wg_s, fsem.at[0]),
                    pltpu.make_async_copy(wu_hbm, wu_s, fsem.at[1]),
                    pltpu.make_async_copy(wd_hbm, wd_s, fsem.at[2]))

        wr_copy = pltpu.make_async_copy(wr_hbm, wr_s, fsem.at[3])

        def layernorm(j, top):
            wr = wr_s[...].astype(_F32).reshape(1, D)

            def slab(i, top):
                t1, t2 = top
                r0 = pl.multiple_of(j * BQ + i * LNR, LNR)
                r = pl.ds(r0, LNR)
                x = x_s[r, :].astype(_F32)
                m = jnp.sum(x, axis=-1, keepdims=True) * (1.0 / D)
                mb = rb(m)
                d = x - mb
                dm = m - mb
                v = jnp.sum(d * d, axis=-1, keepdims=True) * (1.0 / D) - dm * dm
                v = rb(rb(v) + eps)
                inv = recip(rb(v * lax.rsqrt(v)))
                xn = (rb(d) * inv).astype(_BF)
                xn_s[r, :] = xn
                xf = xn.astype(_F32)
                sc = rb(jnp.sum(xf * wr, axis=-1, keepdims=True)) + 0.0
                bits = lax.bitcast_convert_type(sc, jnp.int32)
                key = (bits ^ ((bits >> 31) & 0x7FFFFFFF)) & -65536
                row = r0 + lax.broadcasted_iota(jnp.int32, (LNR, 1), 0)
                key = jnp.where(sc != sc, _IMIN, key | (S - 1 - row))
                for u in range(LNR // 8):
                    k = key[u * 8:(u + 1) * 8]
                    t2 = jnp.maximum(t2, jnp.minimum(t1, k))
                    t1 = jnp.maximum(t1, k)
                return t1, t2

            return lax.fori_loop(0, BQ // LNR, slab, top, unroll=cfg.get("LNU", 1))

        def route(top):
            t1, t2 = top
            k1 = jnp.max(t1)
            k2 = jnp.max(jnp.where(t1 == k1, t2, t1))
            return k1, k2

        def ffn(k1, k2):
            i1, i2 = (S - 1 - (k & 0xFFFF) for k in (k1, k2))

            def score(k):
                kk = jnp.full((16, D), k, jnp.int32) & -65536
                return lax.bitcast_convert_type((kk ^ ((kk >> 31) & 0x7FFFFFFF)) & -65536, _F32)

            m1, m2 = score(k1), score(k2)
            sub = lax.broadcasted_iota(jnp.int32, (16, D), 0)
            grp = []
            for i in (i1, i2):
                base = pl.multiple_of((i // 16) * 16, 16)
                blk = xn_s[pl.ds(base, 16), :]
                grp.append(jnp.where(sub == i - base, blk, jnp.zeros_like(blk)))
            xs = jnp.concatenate(grp, axis=0)
            for c in ffn_copies():
                c.wait()
            gt = rb(silu(rb(jnp.dot(xs, wg_s[...], preferred_element_type=_F32))))
            up = rb(jnp.dot(xs, wu_s[...], preferred_element_type=_F32))
            hid = (gt * up).astype(_BF)
            y = rb(jnp.dot(hid, wd_s[...], preferred_element_type=_F32))
            for k, (i, m) in enumerate(((i1, m1), (i2, m2))):
                upd = rb(y[k * 16:(k + 1) * 16] * rb(sigmoid(m)))
                rs = pl.ds(pl.multiple_of((i // 16) * 16, 16), 16)
                z = (xn_s[rs, :].astype(_F32) + upd).astype(_BF)
                xn_s[rs, :] = jnp.where(sub == i % 16, z, xn_s[rs, :])

        def attention_pair(slot, prefetch):
            def qproj(j):
                q2 = jnp.dot(xn_s[pl.ds(j * BQ, BQ), :], wq_s[slot], preferred_element_type=_F32)
                return (q2 * qscale).astype(_BF)

            RC = cfg.get("RC", 0)
            HO = cfg.get("HO", 0)
            QO = cfg.get("QO", 2)

            def soft(s):
                e = jnp.exp2(s - jnp.max(s, axis=1, keepdims=True))
                return e.astype(_BF), jnp.sum(e, axis=1, keepdims=True)

            def pv(el, h):
                e, l = el
                o = lax.dot_general(vt_s[slot, h], e, _NT, preferred_element_type=_F32)
                if RC == 0:
                    il = jnp.broadcast_to(1.0 / l, (BQ, 128)).T[0:1]
                elif RC == 1:
                    il = 1.0 / jnp.broadcast_to(l, (BQ, 128)).T[0:1]
                elif RC == 2:
                    r0 = pl.reciprocal(l, approx=True)
                    il = jnp.broadcast_to(r0 * (2.0 - l * r0), (BQ, 128)).T[0:1]
                elif RC == 3:
                    lt = jnp.broadcast_to(l, (BQ, 128)).T[0:1]
                    r0 = pl.reciprocal(lt, approx=True)
                    il = r0 * (2.0 - lt * r0)
                return (o * il).astype(_BF)

            if cfg.get('PF', 0) == 0:
                prefetch()
            wot_s[...] = wo_s[slot].T
            q2 = qproj(0)
            if cfg.get('PF', 0) == 1:
                prefetch()
            SK_ = cfg.get("SKEW", 0)
            prev = None

            def oproj(j, ot):
                acc_s[:, pl.ds(j * BQ, BQ)] += jnp.dot(wot_s[...], ot, preferred_element_type=_F32)

            for j in range(NQ):
                last = j + 1 == NQ
                if SK_ == 2 and prev is not None:
                    ss = [jnp.dot(q2[:, 0:256], kp_s[slot, 0], preferred_element_type=_F32)]
                    oproj(*prev)
                    prev = None
                    ss.append(jnp.dot(q2[:, 128:384], kp_s[slot, 1], preferred_element_type=_F32))
                else:
                    ss = [jnp.dot(q2[:, h * 128:h * 128 + 256], kp_s[slot, h], preferred_element_type=_F32)
                          for h in range(2)]
                if SK_ == 1 and prev is not None:
                    oproj(*prev)
                    prev = None
                if QO == 0 and not last:
                    q2 = qproj(j + 1)
                if HO == 0:
                    o0 = pv(soft(ss[0]), 0)
                    if QO == 1 and not last:
                        q2 = qproj(j + 1)
                    o1 = pv(soft(ss[1]), 1)
                else:
                    e0, e1 = soft(ss[0]), soft(ss[1])
                    o0 = pv(e0, 0)
                    if QO == 1 and not last:
                        q2 = qproj(j + 1)
                    o1 = pv(e1, 1)
                ot = jnp.concatenate([o0, o1], axis=0)
                if QO == 2 and not last:
                    q2 = qproj(j + 1)
                if SK_ and not last:
                    prev = (j, ot)
                else:
                    oproj(j, ot)
                if QO == 3 and not last:
                    q2 = qproj(j + 1)

        c0 = pair_copies(0, 0)
        wr_copy.start()
        x_copy(0).start()
        with scope('zero'):
            acc_s[...] = jnp.zeros_like(acc_s)
            zpad = jnp.zeros((256 - DH, W), _BF)
            for sl in range(2):
                kp_s[sl, 0, pl.ds(DH, 256 - DH), :] = zpad
                kp_s[sl, 1, pl.ds(0, 256 - DH), :] = zpad
        wr_copy.wait()
        top = (jnp.full((8, 1), _IMIN, jnp.int32),) * 2
        later = cfg.get("LATER", ((0,), (1, 2), (3,), (4,)))
        with scope('ln'):
            for j in range(NQ):
                x_copy(j).wait()
                if j + 1 < NQ:
                    x_copy(j + 1).start()
                for c in later[j]:
                    c0[c].start()
                top = layernorm(j, top)

        for c in ffn_copies():
            c.start()

        def loop(p, carry):
            slot = p % 2
            for c in pair_copies(p, slot):
                c.wait()

            def prefetch():
                for c in pair_copies(jnp.minimum(p + 1, NP - 1), 1 - slot):
                    c.start()

            attention_pair(slot, prefetch)
            return carry

        with scope('loop'):
            lax.fori_loop(0, NP, loop, 0)
            for c in pair_copies(NP - 1, NP % 2):
                c.wait()
        k1, k2 = route(top)
        i1, i2 = (S - 1 - (k & 0xFFFF) for k in (k1, k2))

        def fslab(r0):
            r = pl.ds(pl.multiple_of(r0, FR), FR)
            sg = acc_s[:, r].T * silu(xn_s[r, :].astype(_F32))
            o_s[r, :] = (x_s[r, :].astype(_F32) + sg).astype(o_s.dtype)

        def routed(j):
            return (i1 // OR == j) | (i2 // OR == j)

        with scope('fin'):
            for j in range(NO):
                for i in range(OR // FR):
                    fslab(j * OR + i * FR)

                @pl.when(jnp.logical_not(routed(j)))
                def _():
                    o_copy(j).start()
        with scope('ffn'):
            ffn(k1, k2)
            fslab(i1 // FR * FR)
            fslab(i2 // FR * FR)
            for j in range(NO):
                @pl.when(routed(j))
                def _():
                    o_copy(j).start()
        with scope('owait'):
            for j in range(NO):
                o_copy(j).wait()

    def hbm(a):
        return pltpu.with_memory_space_constraint(a, pltpu.HBM)

    kt = jnp.swapaxes(A_k_cache, 2, 3)
    vt = jnp.swapaxes(A_v_cache, 2, 3)
    any_spec = pl.BlockSpec(memory_space=pl.ANY)
    DMA = pltpu.SemaphoreType.DMA
    return pl.pallas_call(
        kernel,
        in_specs=[any_spec] * 9,
        out_specs=any_spec,
        out_shape=jax.ShapeDtypeStruct((1, S, D), A_x.dtype),
        scratch_shapes=[
            pltpu.VMEM((S, D), _BF),
            pltpu.VMEM((S, D), _BF),
            pltpu.VMEM((S, D), _BF),
            pltpu.VMEM((D, S), _F32),
            pltpu.VMEM((2, 2, 256, W), _BF),
            pltpu.VMEM((2, 2, DH, W), _BF),
            pltpu.VMEM((2, D, PW), _BF),
            pltpu.VMEM((2, PW, D), _BF),
            pltpu.VMEM((D, PW), _BF),
            pltpu.VMEM((D,), _BF),
            pltpu.VMEM((D, F), _BF),
            pltpu.VMEM((D, F), _BF),
            pltpu.VMEM((F, D), _BF),
            DMA((NQ,)), DMA((2, 5)), DMA((4,)), DMA((NO,)),
        ],
        compiler_params=pltpu.CompilerParams(vmem_limit_bytes=100 * 2**20, flags=cfg.get("flags")),
        name="mykernel",
    )(hbm(A_x), hbm(kt), hbm(vt), hbm(A_wq), hbm(A_wo), hbm(B_w_r),
      hbm(B_w_gate), hbm(B_w_up), hbm(B_w_down))
```

```python
import numpy as np
import jax
import jax.numpy as jnp
from jax import lax
import jax.experimental.pallas as pl
import jax.experimental.pallas.tpu as pltpu

_NT = (((1,), (1,)), ((), ()))
_BF = jnp.bfloat16
_F32 = jnp.float32
_IMIN = -2 ** 31


@jax.jit
def pallas_recurrent_scan__sliding_block_cached__moe_arch_mod__prompt_kernel(
    A_x: jax.Array,
    A_k_cache: jax.Array,
    A_v_cache: jax.Array,
    A_wq: jax.Array,
    A_wo: jax.Array,
    B_x: jax.Array,
    B_w_r: jax.Array,
    B_w_gate: jax.Array,
    B_w_up: jax.Array,
    B_w_down: jax.Array,
):
    del B_x
    _, S, D = A_x.shape
    H, DH = 32, 192
    SK = A_k_cache.shape[2]
    W = min(4096, max(256, SK // 4))
    F = B_w_gate.shape[1]
    NP = H // 2
    PW = 2 * DH
    BQ = 512
    NQ = S // BQ
    OR = 128
    NO = S // OR
    LNR = 128
    FR = OR
    qscale = float(DH ** -0.5 * np.log2(np.e))
    eps = float(np.asarray(1e-5, np.float32).astype(jnp.bfloat16).astype(np.float32))

    def rb(a):
        return a.astype(_BF).astype(_F32)

    def recip(a):
        r0 = pl.reciprocal(a, approx=True)
        return r0 * (2.0 - a * r0)

    def sigmoid(a):
        return 0.5 * jnp.tanh(0.5 * a) + 0.5

    def silu(a):
        h = 0.5 * a
        return h * jnp.tanh(h) + h

    def kernel(x_hbm, kt_hbm, vt_hbm, wq_hbm, wo_hbm, wr_hbm, wg_hbm, wu_hbm, wd_hbm, o_hbm,
               x_s, xn_s, o_s, acc_s, kp_s, vt_s, wq_s, wo_s, wot_s, wr_s,
               wg_s, wu_s, wd_s, xsem, psem, fsem, osem):

        def x_copy(j):
            return pltpu.make_async_copy(x_hbm.at[0, pl.ds(j * BQ, BQ), :], x_s.at[pl.ds(j * BQ, BQ), :], xsem.at[j])

        def o_copy(j):
            return pltpu.make_async_copy(o_s.at[pl.ds(j * OR, OR), :], o_hbm.at[0, pl.ds(j * OR, OR), :], osem.at[j])

        def pair_copies(p, slot):
            win = pl.ds(SK - W, W)
            c0 = pl.multiple_of(p * PW, 128)
            return (
                pltpu.make_async_copy(wq_hbm.at[:, pl.ds(c0, PW)], wq_s.at[slot], psem.at[slot, 0]),
                pltpu.make_async_copy(kt_hbm.at[0, 2 * p, :, win], kp_s.at[slot, 0, pl.ds(0, DH), :], psem.at[slot, 1]),
                pltpu.make_async_copy(kt_hbm.at[0, 2 * p + 1, :, win], kp_s.at[slot, 1, pl.ds(256 - DH, DH), :], psem.at[slot, 2]),
                pltpu.make_async_copy(vt_hbm.at[0, pl.ds(2 * p, 2), :, win], vt_s.at[slot], psem.at[slot, 3]),
                pltpu.make_async_copy(wo_hbm.at[pl.ds(c0, PW), :], wo_s.at[slot], psem.at[slot, 4]),
            )

        def ffn_copies():
            return (pltpu.make_async_copy(wg_hbm, wg_s, fsem.at[0]),
                    pltpu.make_async_copy(wu_hbm, wu_s, fsem.at[1]),
                    pltpu.make_async_copy(wd_hbm, wd_s, fsem.at[2]))

        wr_copy = pltpu.make_async_copy(wr_hbm, wr_s, fsem.at[3])

        def layernorm(j, top):
            wr = wr_s[...].astype(_F32).reshape(1, D)

            def slab(i, top):
                t1, t2 = top
                r0 = pl.multiple_of(j * BQ + i * LNR, LNR)
                r = pl.ds(r0, LNR)
                x = x_s[r, :].astype(_F32)
                m = jnp.sum(x, axis=-1, keepdims=True) * (1.0 / D)
                mb = rb(m)
                d = x - mb
                dm = m - mb
                v = jnp.sum(d * d, axis=-1, keepdims=True) * (1.0 / D) - dm * dm
                v = rb(rb(v) + eps)
                inv = recip(rb(v * lax.rsqrt(v)))
                xn = (rb(d) * inv).astype(_BF)
                xn_s[r, :] = xn
                xf = xn.astype(_F32)
                sc = rb(jnp.sum(xf * wr, axis=-1, keepdims=True)) + 0.0
                bits = lax.bitcast_convert_type(sc, jnp.int32)
                key = (bits ^ ((bits >> 31) & 0x7FFFFFFF)) & -65536
                row = r0 + lax.broadcasted_iota(jnp.int32, (LNR, 1), 0)
                key = jnp.where(sc != sc, _IMIN, key | (S - 1 - row))
                for u in range(LNR // 8):
                    k = key[u * 8:(u + 1) * 8]
                    t2 = jnp.maximum(t2, jnp.minimum(t1, k))
                    t1 = jnp.maximum(t1, k)
                return t1, t2

            return lax.fori_loop(0, BQ // LNR, slab, top, unroll=2)

        def route(top):
            t1, t2 = top
            k1 = jnp.max(t1)
            k2 = jnp.max(jnp.where(t1 == k1, t2, t1))
            return k1, k2

        def ffn(k1, k2):
            i1, i2 = (S - 1 - (k & 0xFFFF) for k in (k1, k2))

            def score(k):
                kk = jnp.full((16, D), k, jnp.int32) & -65536
                return lax.bitcast_convert_type((kk ^ ((kk >> 31) & 0x7FFFFFFF)) & -65536, _F32)

            m1, m2 = score(k1), score(k2)
            sub = lax.broadcasted_iota(jnp.int32, (16, D), 0)
            grp = []
            for i in (i1, i2):
                base = pl.multiple_of((i // 16) * 16, 16)
                blk = xn_s[pl.ds(base, 16), :]
                grp.append(jnp.where(sub == i - base, blk, jnp.zeros_like(blk)))
            xs = jnp.concatenate(grp, axis=0)
            for c in ffn_copies():
                c.wait()
            gt = rb(silu(rb(jnp.dot(xs, wg_s[...], preferred_element_type=_F32))))
            up = rb(jnp.dot(xs, wu_s[...], preferred_element_type=_F32))
            hid = (gt * up).astype(_BF)
            y = rb(jnp.dot(hid, wd_s[...], preferred_element_type=_F32))
            for k, (i, m) in enumerate(((i1, m1), (i2, m2))):
                upd = rb(y[k * 16:(k + 1) * 16] * rb(sigmoid(m)))
                rs = pl.ds(pl.multiple_of((i // 16) * 16, 16), 16)
                z = (xn_s[rs, :].astype(_F32) + upd).astype(_BF)
                xn_s[rs, :] = jnp.where(sub == i % 16, z, xn_s[rs, :])

        def attention_pair(slot, prefetch):
            def qproj(j):
                q2 = jnp.dot(xn_s[pl.ds(j * BQ, BQ), :], wq_s[slot], preferred_element_type=_F32)
                return (q2 * qscale).astype(_BF)

            def attend(s, h):
                e = jnp.exp2(s - jnp.max(s, axis=1, keepdims=True))
                l = jnp.sum(e, axis=1, keepdims=True)
                o = lax.dot_general(vt_s[slot, h], e.astype(_BF), _NT, preferred_element_type=_F32)
                il = jnp.broadcast_to(1.0 / l, (BQ, 128)).T[0:1]
                return (o * il).astype(_BF)

            prefetch()
            wot_s[...] = wo_s[slot].T
            q2 = qproj(0)
            for j in range(NQ):
                ss = [jnp.dot(q2[:, h * 128:h * 128 + 256], kp_s[slot, h], preferred_element_type=_F32)
                      for h in range(2)]
                ot = jnp.concatenate([attend(ss[h], h) for h in range(2)], axis=0)
                if j + 1 < NQ:
                    q2 = qproj(j + 1)
                acc_s[:, pl.ds(j * BQ, BQ)] += jnp.dot(wot_s[...], ot, preferred_element_type=_F32)

        c0 = pair_copies(0, 0)
        wr_copy.start()
        x_copy(0).start()
        acc_s[...] = jnp.zeros_like(acc_s)
        zpad = jnp.zeros((256 - DH, W), _BF)
        for sl in range(2):
            kp_s[sl, 0, pl.ds(DH, 256 - DH), :] = zpad
            kp_s[sl, 1, pl.ds(0, 256 - DH), :] = zpad
        wr_copy.wait()
        top = (jnp.full((8, 1), _IMIN, jnp.int32),) * 2
        later = ((0,), (1, 2), (3,), (4,))
        for j in range(NQ):
            x_copy(j).wait()
            if j + 1 < NQ:
                x_copy(j + 1).start()
            for c in later[j]:
                c0[c].start()
            top = layernorm(j, top)

        for c in ffn_copies():
            c.start()

        def loop(p, carry):
            slot = p % 2
            for c in pair_copies(p, slot):
                c.wait()

            def prefetch():
                for c in pair_copies(jnp.minimum(p + 1, NP - 1), 1 - slot):
                    c.start()

            attention_pair(slot, prefetch)
            return carry

        lax.fori_loop(0, NP, loop, 0)
        for c in pair_copies(NP - 1, NP % 2):
            c.wait()
        k1, k2 = route(top)
        i1, i2 = (S - 1 - (k & 0xFFFF) for k in (k1, k2))

        def fslab(r0):
            r = pl.ds(pl.multiple_of(r0, FR), FR)
            sg = acc_s[:, r].T * silu(xn_s[r, :].astype(_F32))
            o_s[r, :] = (x_s[r, :].astype(_F32) + sg).astype(o_s.dtype)

        def routed(j):
            return (i1 // OR == j) | (i2 // OR == j)

        for j in range(NO):
            for i in range(OR // FR):
                fslab(j * OR + i * FR)

            @pl.when(jnp.logical_not(routed(j)))
            def _():
                o_copy(j).start()
        ffn(k1, k2)
        fslab(i1 // FR * FR)
        fslab(i2 // FR * FR)
        for j in range(NO):
            @pl.when(routed(j))
            def _():
                o_copy(j).start()
        for j in range(NO):
            o_copy(j).wait()

    def hbm(a):
        return pltpu.with_memory_space_constraint(a, pltpu.HBM)

    kt = jnp.swapaxes(A_k_cache, 2, 3)
    vt = jnp.swapaxes(A_v_cache, 2, 3)
    any_spec = pl.BlockSpec(memory_space=pl.ANY)
    DMA = pltpu.SemaphoreType.DMA
    return pl.pallas_call(
        kernel,
        in_specs=[any_spec] * 9,
        out_specs=any_spec,
        out_shape=jax.ShapeDtypeStruct((1, S, D), A_x.dtype),
        scratch_shapes=[
            pltpu.VMEM((S, D), _BF),
            pltpu.VMEM((S, D), _BF),
            pltpu.VMEM((S, D), _BF),
            pltpu.VMEM((D, S), _F32),
            pltpu.VMEM((2, 2, 256, W), _BF),
            pltpu.VMEM((2, 2, DH, W), _BF),
            pltpu.VMEM((2, D, PW), _BF),
            pltpu.VMEM((2, PW, D), _BF),
            pltpu.VMEM((D, PW), _BF),
            pltpu.VMEM((D,), _BF),
            pltpu.VMEM((D, F), _BF),
            pltpu.VMEM((D, F), _BF),
            pltpu.VMEM((F, D), _BF),
            DMA((NQ,)), DMA((2, 5)), DMA((4,)), DMA((NO,)),
        ],
        compiler_params=pltpu.CompilerParams(vmem_limit_bytes=100 * 2**20),
        name="mykernel",
    )(hbm(A_x), hbm(kt), hbm(vt), hbm(A_wq), hbm(A_wo), hbm(B_w_r),
      hbm(B_w_gate), hbm(B_w_up), hbm(B_w_down))
```

```python
import numpy as np
import jax
import jax.numpy as jnp
from jax import lax
import jax.experimental.pallas as pl
import jax.experimental.pallas.tpu as pltpu

_NT = (((1,), (1,)), ((), ()))
_BF = jnp.bfloat16
_F32 = jnp.float32
_IMIN = -2 ** 31


@jax.jit
def pallas_recurrent_scan__sliding_block_cached__moe_arch_mod__prompt_kernel(
    A_x: jax.Array,
    A_k_cache: jax.Array,
    A_v_cache: jax.Array,
    A_wq: jax.Array,
    A_wo: jax.Array,
    B_x: jax.Array,
    B_w_r: jax.Array,
    B_w_gate: jax.Array,
    B_w_up: jax.Array,
    B_w_down: jax.Array,
):
    del B_x
    _, S, D = A_x.shape
    H, DH = 32, 192
    SK = A_k_cache.shape[2]
    W = min(4096, max(256, SK // 4))
    F = B_w_gate.shape[1]
    NP = H // 2
    PW = 2 * DH
    BQ = 512
    NQ = S // BQ
    AB = 256
    OR = 128
    NO = S // OR
    LNR = 128
    FR = OR
    qscale = float(DH ** -0.5 * np.log2(np.e))
    eps = float(np.asarray(1e-5, np.float32).astype(jnp.bfloat16).astype(np.float32))

    def rb(a):
        return a.astype(_BF).astype(_F32)

    def recip(a):
        r0 = pl.reciprocal(a, approx=True)
        return r0 * (2.0 - a * r0)

    def sigmoid(a):
        return 0.5 * jnp.tanh(0.5 * a) + 0.5

    def silu(a):
        h = 0.5 * a
        return h * jnp.tanh(h) + h

    def kernel(x_hbm, kt_hbm, vt_hbm, wq_hbm, wo_hbm, wr_hbm, wg_hbm, wu_hbm, wd_hbm, o_hbm,
               x_s, xn_s, o_s, acc_s, kp_s, vt_s, wq_s, wo_s, wot_s, wr_s,
               wg_s, wu_s, wd_s, xsem, psem, fsem, osem):

        def x_copy(j):
            return pltpu.make_async_copy(x_hbm.at[0, pl.ds(j * BQ, BQ), :], x_s.at[pl.ds(j * BQ, BQ), :], xsem.at[j])

        def o_copy(j):
            return pltpu.make_async_copy(o_s.at[pl.ds(j * OR, OR), :], o_hbm.at[0, pl.ds(j * OR, OR), :], osem.at[j])

        def pair_copies(p, slot):
            win = pl.ds(SK - W, W)
            c0 = pl.multiple_of(p * PW, 128)
            return (
                pltpu.make_async_copy(wq_hbm.at[:, pl.ds(c0, PW)], wq_s.at[slot], psem.at[slot, 0]),
                pltpu.make_async_copy(kt_hbm.at[0, 2 * p, :, win], kp_s.at[slot, 0, pl.ds(0, DH), :], psem.at[slot, 1]),
                pltpu.make_async_copy(kt_hbm.at[0, 2 * p + 1, :, win], kp_s.at[slot, 1, pl.ds(256 - DH, DH), :], psem.at[slot, 2]),
                pltpu.make_async_copy(vt_hbm.at[0, pl.ds(2 * p, 2), :, win], vt_s.at[slot], psem.at[slot, 3]),
                pltpu.make_async_copy(wo_hbm.at[pl.ds(c0, PW), :], wo_s.at[slot], psem.at[slot, 4]),
            )

        def ffn_copies():
            return (pltpu.make_async_copy(wg_hbm, wg_s, fsem.at[0]),
                    pltpu.make_async_copy(wu_hbm, wu_s, fsem.at[1]),
                    pltpu.make_async_copy(wd_hbm, wd_s, fsem.at[2]))

        wr_copy = pltpu.make_async_copy(wr_hbm, wr_s, fsem.at[3])

        def layernorm(j, top):
            wr = wr_s[...].astype(_F32).reshape(1, D)

            def slab(i, top):
                t1, t2 = top
                r0 = pl.multiple_of(j * BQ + i * LNR, LNR)
                r = pl.ds(r0, LNR)
                x = x_s[r, :].astype(_F32)
                m = jnp.sum(x, axis=-1, keepdims=True) * (1.0 / D)
                mb = rb(m)
                d = x - mb
                dm = m - mb
                v = jnp.sum(d * d, axis=-1, keepdims=True) * (1.0 / D) - dm * dm
                v = rb(rb(v) + eps)
                inv = recip(rb(v * lax.rsqrt(v)))
                xn = (rb(d) * inv).astype(_BF)
                xn_s[r, :] = xn
                xf = xn.astype(_F32)
                sc = rb(jnp.sum(xf * wr, axis=-1, keepdims=True)) + 0.0
                bits = lax.bitcast_convert_type(sc, jnp.int32)
                key = (bits ^ ((bits >> 31) & 0x7FFFFFFF)) & -65536
                row = r0 + lax.broadcasted_iota(jnp.int32, (LNR, 1), 0)
                key = jnp.where(sc != sc, _IMIN, key | (S - 1 - row))
                for u in range(LNR // 8):
                    k = key[u * 8:(u + 1) * 8]
                    t2 = jnp.maximum(t2, jnp.minimum(t1, k))
                    t1 = jnp.maximum(t1, k)
                return t1, t2

            return lax.fori_loop(0, BQ // LNR, slab, top, unroll=2)

        def route(top):
            t1, t2 = top
            k1 = jnp.max(t1)
            k2 = jnp.max(jnp.where(t1 == k1, t2, t1))
            return k1, k2

        def ffn(k1, k2):
            i1, i2 = (S - 1 - (k & 0xFFFF) for k in (k1, k2))

            def score(k):
                kk = jnp.full((16, D), k, jnp.int32) & -65536
                return lax.bitcast_convert_type((kk ^ ((kk >> 31) & 0x7FFFFFFF)) & -65536, _F32)

            m1, m2 = score(k1), score(k2)
            sub = lax.broadcasted_iota(jnp.int32, (16, D), 0)
            grp = []
            for i in (i1, i2):
                base = pl.multiple_of((i // 16) * 16, 16)
                blk = xn_s[pl.ds(base, 16), :]
                grp.append(jnp.where(sub == i - base, blk, jnp.zeros_like(blk)))
            xs = jnp.concatenate(grp, axis=0)
            for c in ffn_copies():
                c.wait()
            gt = rb(silu(rb(jnp.dot(xs, wg_s[...], preferred_element_type=_F32))))
            up = rb(jnp.dot(xs, wu_s[...], preferred_element_type=_F32))
            hid = (gt * up).astype(_BF)
            y = rb(jnp.dot(hid, wd_s[...], preferred_element_type=_F32))
            for k, (i, m) in enumerate(((i1, m1), (i2, m2))):
                upd = rb(y[k * 16:(k + 1) * 16] * rb(sigmoid(m)))
                rs = pl.ds(pl.multiple_of((i // 16) * 16, 16), 16)
                z = (xn_s[rs, :].astype(_F32) + upd).astype(_BF)
                xn_s[rs, :] = jnp.where(sub == i % 16, z, xn_s[rs, :])

        def attention_pair(slot, prefetch):
            def qproj(j):
                q2 = jnp.dot(xn_s[pl.ds(j * BQ, BQ), :], wq_s[slot], preferred_element_type=_F32)
                return (q2 * qscale).astype(_BF)

            def attend(s, h):
                e = jnp.exp2(s - jnp.max(s, axis=1, keepdims=True))
                l = jnp.sum(e, axis=1, keepdims=True)
                o = lax.dot_general(vt_s[slot, h], e.astype(_BF), _NT, preferred_element_type=_F32)
                il = jnp.broadcast_to(recip(l), (AB, 128)).T[0:1]
                return (o * il).astype(_BF)

            prefetch()
            wot_s[...] = wo_s[slot].T
            q2 = jnp.concatenate([qproj(j) for j in range(NQ)], axis=0)
            ots = []
            for u in range(S // AB):
                qq = q2[u * AB:(u + 1) * AB]
                ss = [jnp.dot(qq[:, h * 128:h * 128 + 256], kp_s[slot, h], preferred_element_type=_F32)
                      for h in range(2)]
                ots.append(jnp.concatenate([attend(ss[h], h) for h in range(2)], axis=0))
            acc_s[...] += jnp.dot(wot_s[...], jnp.concatenate(ots, axis=1), preferred_element_type=_F32)

        c0 = pair_copies(0, 0)
        wr_copy.start()
        x_copy(0).start()
        acc_s[...] = jnp.zeros_like(acc_s)
        zpad = jnp.zeros((256 - DH, W), _BF)
        for sl in range(2):
            kp_s[sl, 0, pl.ds(DH, 256 - DH), :] = zpad
            kp_s[sl, 1, pl.ds(0, 256 - DH), :] = zpad
        wr_copy.wait()
        top = (jnp.full((8, 1), _IMIN, jnp.int32),) * 2
        later = ((0,), (1, 2), (3,), (4,))
        for j in range(NQ):
            x_copy(j).wait()
            if j + 1 < NQ:
                x_copy(j + 1).start()
            for c in later[j]:
                c0[c].start()
            top = layernorm(j, top)

        for c in ffn_copies():
            c.start()

        def loop(p, carry):
            slot = p % 2
            for c in pair_copies(p, slot):
                c.wait()

            def prefetch():
                for c in pair_copies(jnp.minimum(p + 1, NP - 1), 1 - slot):
                    c.start()

            attention_pair(slot, prefetch)
            return carry

        lax.fori_loop(0, NP, loop, 0)
        for c in pair_copies(NP - 1, NP % 2):
            c.wait()
        k1, k2 = route(top)
        i1, i2 = (S - 1 - (k & 0xFFFF) for k in (k1, k2))

        def fslab(r0):
            r = pl.ds(pl.multiple_of(r0, FR), FR)
            sg = acc_s[:, r].T * silu(xn_s[r, :].astype(_F32))
            o_s[r, :] = (x_s[r, :].astype(_F32) + sg).astype(o_s.dtype)

        def routed(j):
            return (i1 // OR == j) | (i2 // OR == j)

        for j in range(NO):
            for i in range(OR // FR):
                fslab(j * OR + i * FR)

            @pl.when(jnp.logical_not(routed(j)))
            def _():
                o_copy(j).start()
        ffn(k1, k2)
        fslab(i1 // FR * FR)
        fslab(i2 // FR * FR)
        for j in range(NO):
            @pl.when(routed(j))
            def _():
                o_copy(j).start()
        for j in range(NO):
            o_copy(j).wait()

    def hbm(a):
        return pltpu.with_memory_space_constraint(a, pltpu.HBM)

    kt = jnp.swapaxes(A_k_cache, 2, 3)
    vt = jnp.swapaxes(A_v_cache, 2, 3)
    any_spec = pl.BlockSpec(memory_space=pl.ANY)
    DMA = pltpu.SemaphoreType.DMA
    return pl.pallas_call(
        kernel,
        in_specs=[any_spec] * 9,
        out_specs=any_spec,
        out_shape=jax.ShapeDtypeStruct((1, S, D), A_x.dtype),
        scratch_shapes=[
            pltpu.VMEM((S, D), _BF),
            pltpu.VMEM((S, D), _BF),
            pltpu.VMEM((S, D), _BF),
            pltpu.VMEM((D, S), _F32),
            pltpu.VMEM((2, 2, 256, W), _BF),
            pltpu.VMEM((2, 2, DH, W), _BF),
            pltpu.VMEM((2, D, PW), _BF),
            pltpu.VMEM((2, PW, D), _BF),
            pltpu.VMEM((D, PW), _BF),
            pltpu.VMEM((D,), _BF),
            pltpu.VMEM((D, F), _BF),
            pltpu.VMEM((D, F), _BF),
            pltpu.VMEM((F, D), _BF),
            DMA((NQ,)), DMA((2, 5)), DMA((4,)), DMA((NO,)),
        ],
        compiler_params=pltpu.CompilerParams(vmem_limit_bytes=100 * 2**20),
        name="mykernel",
    )(hbm(A_x), hbm(kt), hbm(vt), hbm(A_wq), hbm(A_wo), hbm(B_w_r),
      hbm(B_w_gate), hbm(B_w_up), hbm(B_w_down))
```
